```python
import jax
import jax.numpy as jnp

def _softmax(x, axis=-1):
    return jax.nn.softmax(x, axis=axis)
def _gelu(x):
    return jax.nn.gelu(x, approximate=True)
def _silu(x):
    return jax.nn.silu(x)
def _sigmoid(x):
    return jax.nn.sigmoid(x)
def _layernorm(x, axis=-1, eps=1e-5):
    m = jnp.mean(x, axis=axis, keepdims=True)
    v = jnp.var(x, axis=axis, keepdims=True)
    return (x - m) / jnp.sqrt(v + eps)
def _scatter_add(tgt, idx, src, axis=0):
    return tgt.at[idx].add(src)
def _segment_sum(src, seg, n):
    return jax.ops.segment_sum(src, seg, n)
class _Rng:
    def __init__(self, key):
        self._k = key
    def _next(self):
        self._k, sub = jax.random.split(self._k)
        return sub
    def normal(self, shape):
        return jax.random.normal(self._next(), shape, dtype=jnp.bfloat16)
    def randint(self, lo, hi, shape):
        return jax.random.randint(self._next(), shape, lo, hi, dtype=jnp.int32)
    def uniform(self, shape, lo=0.0, hi=1.0):
        return jax.random.uniform(self._next(), shape, jnp.bfloat16, lo, hi)
    def permutation(self, n):
        return jax.random.permutation(self._next(), n)


kernel_name = 'interleave_layers__softmax_full_mha__ssm_conv_h3__prompt'

def setup_inputs():
    _rng = _Rng(jax.random.key(int.from_bytes(__import__("os").urandom(4), "little")))
    _w = (lambda a: (lambda t: t.astype(jnp.bfloat16) if jnp.issubdtype(t.dtype, jnp.floating) else t)(jnp.asarray(a)))
    def _A_setup():
        B, S, D = 1, 2048, 1024
        return {
            "x": _w((lambda *s: _rng.normal(s) * 0.05)(B, S, D)),
            "wqkv": _w((lambda *s: _rng.normal(s) * 0.05)(D, 3 * D)),
            "wo": _w((lambda *s: _rng.normal(s) * 0.05)(D, D)),
        }
    _A_in = _A_setup()

    def _B_setup():
        B, S, D = 1, 2048, 1024
        ks = 4
        return {
            "q": _w((lambda *s: _rng.normal(s) * 0.05)(B, S, D)),
            "k": _w((lambda *s: _rng.normal(s) * 0.05)(B, S, D)),
            "v": _w((lambda *s: _rng.normal(s) * 0.05)(B, S, D)),
            "shift_k": _w((lambda *s: _rng.normal(s) * 0.05)(D, ks) * 0.5),
            "ssm_k": _w((lambda *s: _rng.normal(s) * 0.05)(D, S) * (1.0 / S ** 0.5)),
            "ssm_D": _w((lambda *s: _rng.normal(s) * 0.05)(D)),
        }
    _B_in = _B_setup()

    return {
        "A_x": _A_in["x"],
        "A_wqkv": _A_in["wqkv"],
        "A_wo": _A_in["wo"],
        "B_q": _B_in["q"],
        "B_k": _B_in["k"],
        "B_v": _B_in["v"],
        "B_shift_k": _B_in["shift_k"],
        "B_ssm_k": _B_in["ssm_k"],
        "B_ssm_D": _B_in["ssm_D"],
    }

def reference(A_x, A_wqkv, A_wo, B_q, B_k, B_v, B_shift_k, B_ssm_k, B_ssm_D):
    def _A_ref(x, wqkv, wo):
        B, S, D = x.shape
        H = 32; Dh = D // H
        qkv = (lambda x, *d: x.transpose(*d))((x @ wqkv).reshape(B, S, 3, H, Dh), 2, 0, 3, 1, 4)
        q, k, v = qkv[0], qkv[1], qkv[2]
        scale = Dh ** -0.5
        scores = jnp.einsum("bhqd,bhkd->bhqk", q, k) * scale
        p = _softmax(scores, axis=-1)
        o = jnp.einsum("bhqk,bhkd->bhqd", p, v)
        return (lambda x, *d: x.transpose(*d))(o, 0, 2, 1, 3).reshape(B, S, D) @ wo

    def _B_ref(q, k, v, shift_k, ssm_k, ssm_D):
        B, S, D = q.shape
        ks = shift_k.shape[-1]
        k_pad = jnp.pad(k, ((0, 0), (ks - 1, 0), (0, 0)))
        k_shift = jnp.zeros_like(k)
        for t in range(ks):
            k_shift = k_shift + k_pad[:, t:t + S, :] * shift_k[:, ks - 1 - t][None, None, :]
        kv = k_shift * v
        L = 2 * S
        kv_pad = jnp.pad(kv, ((0, 0), (0, S), (0, 0)))
        kf_pad = jnp.pad(ssm_k, ((0, 0), (0, S)))
        kv_f = (lambda x, axes=(-2,-1): jnp.fft.rfft2(x.astype(jnp.float32), axes=axes))(kv_pad[:, None, :, :], axes=(1, 2))
        kf_f = (lambda x, axes=(-2,-1): jnp.fft.rfft2(x.astype(jnp.float32), axes=axes))(kf_pad[:, None, :], axes=(1, 2))
        kf_f = (lambda x, *d: x.transpose(*d))(kf_f, 1, 2, 0)
        y_f = kv_f * kf_f[None, :, :, :]
        y = (lambda x, s, axes=(-2,-1): jnp.fft.irfft2(x, s=s, axes=axes).astype(jnp.bfloat16))(y_f, (1, L), axes=(1, 2))[:, 0, :S, :]
        y = y + kv * ssm_D[None, None, :]
        return q * y

    x = A_x
    x = x + _A_ref(_layernorm(x, axis=-1), A_wqkv, A_wo)
    x = x + _B_ref(_layernorm(x, axis=-1), B_k, B_v, B_shift_k, B_ssm_k, B_ssm_D)
    x = x + _A_ref(_layernorm(x, axis=-1), A_wqkv, A_wo)
    x = x + _B_ref(_layernorm(x, axis=-1), B_k, B_v, B_shift_k, B_ssm_k, B_ssm_D)
    return x
```

```python
import math

import jax
import jax.numpy as jnp
import jax.experimental.pallas as pl
import jax.experimental.pallas.tpu as pltpu

F32 = jnp.float32
BF16 = jnp.bfloat16

S = 2048
D = 1024
DH = 32
NG = D // 128
BM = 256
NB = S // BM
BQ = 512
BK = 128
NQ = S // BQ
NKC = S // BK
C = 128
NC = S // C
EPS = 1e-5
Q_SCALE = DH ** -0.5 * math.log2(math.e)

NT = (((1,), (1,)), ((), ()))


def _layernorm(x):
    m = jnp.mean(x, axis=-1, keepdims=True)
    xc = x - m
    v = jnp.mean(xc * xc, axis=-1, keepdims=True)
    return xc * jax.lax.rsqrt(v + EPS)


def _kernel(x_hbm, wqkv_hbm, wo_hbm, bk_hbm, bv_hbm, sk_ref, ssmk_hbm, ssmd_ref,
            out_hbm,
            xf, xb, wqkv, wo, q, k, vt, s_a, s_b, ot, ck, cv, cs, kpad,
            uf, kf, yf, fmat, gmat, sem_x, sem_w, sem_c, sem_o):

    def x_copy(i):
        r = pl.ds(i * BM, BM)
        return pltpu.make_async_copy(x_hbm.at[r], xb.at[r], sem_x.at[i])

    def w_copy(j):
        if j < 3:
            c = pl.ds(j * D, D)
            return pltpu.make_async_copy(wqkv_hbm.at[:, c], wqkv.at[j], sem_w.at[j])
        return pltpu.make_async_copy(wo_hbm, wo, sem_w.at[3])

    def c_copies(g):
        c = pl.ds(g * 128, 128)
        return (pltpu.make_async_copy(bk_hbm.at[:, c], ck.at[g], sem_c.at[3 * g]),
                pltpu.make_async_copy(bv_hbm.at[:, c], cv.at[g], sem_c.at[3 * g + 1]),
                pltpu.make_async_copy(ssmk_hbm.at[c], cs.at[g], sem_c.at[3 * g + 2]))

    def o_copy(i):
        r = pl.ds(i * BM, BM)
        return pltpu.make_async_copy(xb.at[r], out_hbm.at[r], sem_o.at[i])

    x_copy(0).start()
    for cp in c_copies(0):
        cp.start()
    for j in range(3):
        w_copy(j).start()
    for i in range(1, NB):
        x_copy(i).start()
        for cp in c_copies(i):
            cp.start()
    w_copy(3).start()

    row = jax.lax.broadcasted_iota(jnp.int32, (C, C), 0)
    col = jax.lax.broadcasted_iota(jnp.int32, (C, C), 1)

    def twiddle(r, t):
        f = jnp.where(r < C // 2, 2 * r, 2 * r - (C - 1))
        ph = (((2 * f + 1) * t) & (4 * C - 1)).astype(F32) * (2 * math.pi / (4 * C))
        return jnp.cos(ph), -jnp.sin(ph)

    cr, ci = twiddle(row, col)
    fmat[0:C, :] = cr.astype(BF16)
    fmat[C:2 * C, :] = ci.astype(BF16)
    cr, ci = twiddle(col, row)
    gmat[:, 0:C] = cr.astype(BF16)
    gmat[:, C:2 * C] = ci.astype(BF16)
    kpad[0:8, :] = jnp.zeros((8, 128), F32)

    def project(xn, r0, fillers):
        for j in range(3):
            y = jnp.dot(xn, wqkv[j], preferred_element_type=F32)
            if j == 0:
                y = (y * Q_SCALE).astype(BF16)
                for g in range(NG):
                    q[g, pl.ds(r0, BM), :] = y[:, g * 128:(g + 1) * 128]
            elif j == 1:
                y = y.astype(BF16)
                for g in range(NG):
                    k[g, pl.ds(r0, BM), :] = y[:, g * 128:(g + 1) * 128]
            else:
                vt[:, pl.ds(r0, BM)] = y.T.astype(BF16)
            fillers[j]()

    def conv_forward(g):
        lanes = pl.ds(pl.multiple_of(g * 128, 128), 128)
        sk = sk_ref[:, lanes].astype(F32)
        kpad[8:8 + S, :] = ck[g].astype(F32)
        fm = fmat[...]
        prev = None
        for c in range(NC):
            ks = kpad[8 + c * C:8 + (c + 1) * C, :] * sk[0:1]
            for j in range(1, 4):
                ks = ks + kpad[8 - j + c * C:8 - j + (c + 1) * C, :] * sk[j:j + 1]
            kv = (ks * cv[g, c * C:(c + 1) * C, :].astype(F32)).astype(BF16)
            cv[g, c * C:(c + 1) * C, :] = kv
            uf[c] = jnp.dot(fm, kv, preferred_element_type=F32)
            kc = jax.lax.dot_general(fm, cs[g, :, c * C:(c + 1) * C], NT,
                                     preferred_element_type=F32) * (1.0 / C)
            if prev is None:
                kf[c] = kc
            else:
                h = C // 2
                kf[c, 0:h] = kc[0:h] - prev[C:C + h]
                kf[c, h:C] = kc[h:C] + prev[C + h:2 * C]
                kf[c, C:C + h] = kc[C:C + h] + prev[0:h]
                kf[c, C + h:2 * C] = kc[C + h:2 * C] - prev[h:C]
            prev = kc

    FB = 32

    def conv_mac(chunks):
        def run():
            for c in chunks:
                for fb in range(C // FB):
                    re = slice(fb * FB, (fb + 1) * FB)
                    im = slice(C + fb * FB, C + (fb + 1) * FB)
                    ar = ai = None
                    for j in range(c + 1):
                        kr, ki = kf[j, re], kf[j, im]
                        ur, ui = uf[c - j, re], uf[c - j, im]
                        tr = kr * ur - ki * ui
                        ti = kr * ui + ki * ur
                        ar = tr if ar is None else ar + tr
                        ai = ti if ai is None else ai + ti
                    yf[c, re] = ar.astype(BF16)
                    yf[c, im] = ai.astype(BF16)
        return run

    def conv_inverse(g):
        lanes = pl.ds(pl.multiple_of(g * 128, 128), 128)
        dd = ssmd_ref[:, lanes].astype(F32)
        gm = gmat[...]
        for c in range(NC):
            r = slice(c * C, (c + 1) * C)
            y = jnp.dot(gm, yf[c], preferred_element_type=F32)
            ck[g, r, :] = (y + cv[g, r, :].astype(F32) * dd).astype(BF16)

    def first_body(i, _):
        r0 = pl.multiple_of(i * BM, BM)
        x_copy(i).wait()
        for cp in c_copies(i):
            cp.wait()

        @pl.when(i == 0)
        def _():
            for j in range(3):
                w_copy(j).wait()

        x = xb[pl.ds(r0, BM), :].astype(F32)
        xf[pl.ds(r0, BM), :] = x
        xn = _layernorm(x).astype(BF16)
        conv_forward(i)
        project(xn, r0, (conv_mac(range(0, 9)), conv_mac(range(9, 13)),
                         conv_mac(range(13, NC))))
        conv_inverse(i)
        return 0

    def mix_rows(r0):
        rows = pl.ds(r0, BM)
        x = xf[rows, :] + jnp.dot(xb[rows, :], wo[...], preferred_element_type=F32)
        y = jnp.concatenate([ck[g, rows, :] for g in range(NG)], axis=1)
        return x + _layernorm(x) * y.astype(F32)

    def mid_body(i, _):
        r0 = pl.multiple_of(i * BM, BM)
        x = mix_rows(r0)
        xf[pl.ds(r0, BM), :] = x
        nop = lambda: None
        project(_layernorm(x).astype(BF16), r0, (nop, nop, nop))
        return 0

    def last_body(i, _):
        r0 = pl.multiple_of(i * BM, BM)
        xb[pl.ds(r0, BM), :] = mix_rows(r0).astype(BF16)
        o_copy(i).start()
        return 0

    lane = jax.lax.broadcasted_iota(jnp.int32, (BQ, 128), 1)

    def attn_step(ga, qa, ha, gb, hb, sw, sr, m_prev):
        qq = q[ga, pl.ds(pl.multiple_of(qa * BQ, BQ), BQ), :]
        qm = jnp.where((lane >= ha * DH) & (lane < (ha + 1) * DH), qq, jnp.zeros_like(qq))
        vrows = pl.ds(pl.multiple_of(gb * 128 + hb * DH, DH), DH)
        m = l = acc = None
        for c in range(NKC):
            r = slice(c * BK, (c + 1) * BK)
            s = jax.lax.dot_general(k[ga, r, :], qm, NT, preferred_element_type=F32)
            sw[r, :] = s
            mc = s.reshape(BK // 8, 8, BQ).max(axis=0)
            m = mc if m is None else jnp.maximum(m, mc)
            p = jnp.exp2(sr[r, :] - m_prev)
            lc = p.reshape(BK // 8, 8, BQ).sum(axis=0)
            l = lc if l is None else l + lc
            o = jnp.dot(vt[vrows, r], p.astype(BF16), preferred_element_type=F32)
            acc = o if acc is None else acc + o
        l = jnp.sum(l, axis=0, keepdims=True)
        ot[hb * DH:(hb + 1) * DH, :] = acc / l
        return jnp.max(m, axis=0, keepdims=True)

    def attn_flush(t):
        g, qb = t // NQ, t % NQ
        xb[pl.ds(pl.multiple_of(qb * BQ, BQ), BQ),
           pl.ds(pl.multiple_of(g * 128, 128), 128)] = ot[...].T.astype(BF16)

    def attn_body(t, m):
        tp = jnp.maximum(t - 1, 0)
        g, qb = t // NQ, t % NQ
        m = attn_step(g, qb, 0, tp // NQ, 3, s_a, s_b, m)
        attn_flush(tp)
        m = attn_step(g, qb, 1, g, 0, s_b, s_a, m)
        m = attn_step(g, qb, 2, g, 1, s_a, s_b, m)
        m = attn_step(g, qb, 3, g, 2, s_b, s_a, m)
        return m

    def attn_tail(m):
        g = NG - 1
        l = acc = None
        for c in range(NKC):
            r = slice(c * BK, (c + 1) * BK)
            p = jnp.exp2(s_b[r, :] - m)
            lc = p.reshape(BK // 8, 8, BQ).sum(axis=0)
            l = lc if l is None else l + lc
            o = jnp.dot(vt[g * 128 + 3 * DH:(g + 1) * 128, r], p.astype(BF16),
                        preferred_element_type=F32)
            acc = o if acc is None else acc + o
        ot[3 * DH:, :] = acc / jnp.sum(l, axis=0, keepdims=True)
        xb[S - BQ:, g * 128:] = ot[...].T.astype(BF16)

    s_b[...] = jnp.zeros_like(s_b)
    ot[...] = jnp.zeros_like(ot)

    def layer_body(layer, _):
        @pl.when(layer == 0)
        def _():
            jax.lax.fori_loop(0, NB, first_body, 0)
            w_copy(3).wait()

        m = jax.lax.fori_loop(0, NG * NQ, attn_body, jnp.full((1, BQ), 1e30, F32))
        attn_tail(m)

        @pl.when(layer == 0)
        def _():
            jax.lax.fori_loop(0, NB, mid_body, 0)

        @pl.when(layer == 1)
        def _():
            jax.lax.fori_loop(0, NB, last_body, 0)

        return 0

    jax.lax.fori_loop(0, 2, layer_body, 0)
    for i in range(NB):
        o_copy(i).wait()


@jax.jit
def pallas_interleave_layers__softmax_full_mha__ssm_conv_h3__prompt_kernel(
    A_x: jax.Array,
    A_wqkv: jax.Array,
    A_wo: jax.Array,
    B_q: jax.Array,
    B_k: jax.Array,
    B_v: jax.Array,
    B_shift_k: jax.Array,
    B_ssm_k: jax.Array,
    B_ssm_D: jax.Array,
):
    del B_q
    hbm = pl.BlockSpec(memory_space=pl.ANY)
    vmem = pl.BlockSpec(memory_space=pltpu.VMEM)
    out = pl.pallas_call(
        _kernel,
        out_shape=jax.ShapeDtypeStruct((S, D), BF16),
        in_specs=[hbm, hbm, hbm, hbm, hbm, vmem, hbm, vmem],
        out_specs=hbm,
        scratch_shapes=[
            pltpu.VMEM((S, D), F32),
            pltpu.VMEM((S, D), BF16),
            pltpu.VMEM((3, D, D), BF16),
            pltpu.VMEM((D, D), BF16),
            pltpu.VMEM((NG, S, 128), BF16),
            pltpu.VMEM((NG, S, 128), BF16),
            pltpu.VMEM((D, S), BF16),
            pltpu.VMEM((S, BQ), F32),
            pltpu.VMEM((S, BQ), F32),
            pltpu.VMEM((128, BQ), F32),
            pltpu.VMEM((NG, S, 128), BF16),
            pltpu.VMEM((NG, S, 128), BF16),
            pltpu.VMEM((NG, 128, S), BF16),
            pltpu.VMEM((8 + S, 128), F32),
            pltpu.VMEM((NC, 2 * C, 128), F32),
            pltpu.VMEM((NC, 2 * C, 128), F32),
            pltpu.VMEM((NC, 2 * C, 128), BF16),
            pltpu.VMEM((2 * C, C), BF16),
            pltpu.VMEM((C, 2 * C), BF16),
            pltpu.SemaphoreType.DMA((NB,)),
            pltpu.SemaphoreType.DMA((4,)),
            pltpu.SemaphoreType.DMA((3 * NG,)),
            pltpu.SemaphoreType.DMA((NB,)),
        ],
        compiler_params=pltpu.CompilerParams(vmem_limit_bytes=100 * 2**20),
    )(A_x.reshape(S, D), A_wqkv, A_wo, B_k.reshape(S, D), B_v.reshape(S, D),
      B_shift_k.T, B_ssm_k, B_ssm_D.reshape(1, D))
    return out.reshape(1, S, D)
```

```python
import math

import jax
import jax.numpy as jnp
import jax.experimental.pallas as pl
import jax.experimental.pallas.tpu as pltpu

F32 = jnp.float32
BF16 = jnp.bfloat16

S = 2048
D = 1024
DH = 32
NG = D // 128
BM = 256
NB = S // BM
BQ = 512
BK = 128
NQ = S // BQ
NKC = S // BK
SKEW = 2
C = 128
NC = S // C
EPS = 1e-5
Q_SCALE = DH ** -0.5 * math.log2(math.e)

NT = (((1,), (1,)), ((), ()))


def _layernorm(x):
    m = jnp.mean(x, axis=-1, keepdims=True)
    xc = x - m
    v = jnp.mean(xc * xc, axis=-1, keepdims=True)
    return xc * jax.lax.rsqrt(v + EPS)


def _kernel(x_hbm, wqkv_hbm, wo_hbm, bk_hbm, bv_hbm, sk_ref, ssmk_hbm, ssmd_ref,
            out_hbm,
            xf, xb, wqkv, wo, q, k, vt, s_a, s_b, ot, ck, cv, cs, kpad,
            xnb, uf, kf, yf, fmat, gmat, sem_x, sem_w, sem_c, sem_o):

    def x_copy(i):
        r = pl.ds(i * BM, BM)
        return pltpu.make_async_copy(x_hbm.at[r], xb.at[r], sem_x.at[i])

    def w_copy(j):
        if j < 3:
            c = pl.ds(j * D, D)
            return pltpu.make_async_copy(wqkv_hbm.at[:, c], wqkv.at[j], sem_w.at[j])
        return pltpu.make_async_copy(wo_hbm, wo, sem_w.at[3])

    def c_copies(g):
        c = pl.ds(g * 128, 128)
        return (pltpu.make_async_copy(bk_hbm.at[:, c], ck.at[g], sem_c.at[3 * g]),
                pltpu.make_async_copy(bv_hbm.at[:, c], cv.at[g], sem_c.at[3 * g + 1]),
                pltpu.make_async_copy(ssmk_hbm.at[c], cs.at[g], sem_c.at[3 * g + 2]))

    def o_copy(i):
        r = pl.ds(i * BM, BM)
        return pltpu.make_async_copy(xb.at[r], out_hbm.at[r], sem_o.at[i])

    for i in range(NB):
        x_copy(i).start()
    for j in range(3):
        w_copy(j).start()
    for i in range(NB):
        for cp in c_copies(i):
            cp.start()
    w_copy(3).start()

    row = jax.lax.broadcasted_iota(jnp.int32, (C, C), 0)
    col = jax.lax.broadcasted_iota(jnp.int32, (C, C), 1)

    def twiddle(r, t):
        f = jnp.where(r < C // 2, 2 * r, 2 * r - (C - 1))
        ph = (((2 * f + 1) * t) & (4 * C - 1)).astype(F32) * (2 * math.pi / (4 * C))
        return jnp.cos(ph), -jnp.sin(ph)

    cr, ci = twiddle(row, col)
    fmat[0:C, :] = cr.astype(BF16)
    fmat[C:2 * C, :] = ci.astype(BF16)
    cr, ci = twiddle(col, row)
    gmat[:, 0:C] = cr.astype(BF16)
    gmat[:, C:2 * C] = ci.astype(BF16)
    kpad[0:8, :] = jnp.zeros((8, 128), F32)

    def project(xn, r0, fill):
        for j in range(3):
            for n in range(2):
                y = jnp.dot(xn, wqkv[j, :, n * 512:(n + 1) * 512], preferred_element_type=F32)
                fill(2 * j + n)
                if j == 2:
                    vt[n * 512:(n + 1) * 512, pl.ds(r0, BM)] = y.T.astype(BF16)
                else:
                    y = (y * Q_SCALE if j == 0 else y).astype(BF16)
                    for g in range(4):
                        (q, k)[j][4 * n + g, pl.ds(r0, BM), :] = y[:, g * 128:(g + 1) * 128]

    def conv_forward(g):
        lanes = pl.ds(pl.multiple_of(g * 128, 128), 128)
        sk = sk_ref[:, lanes].astype(F32)
        kpad[8:8 + S, :] = ck[g].astype(F32)
        fm = fmat[...]
        prev = None
        for c in range(NC):
            ks = kpad[8 + c * C:8 + (c + 1) * C, :] * sk[0:1]
            for j in range(1, 4):
                ks = ks + kpad[8 - j + c * C:8 - j + (c + 1) * C, :] * sk[j:j + 1]
            kv = (ks * cv[g, c * C:(c + 1) * C, :].astype(F32)).astype(BF16)
            cv[g, c * C:(c + 1) * C, :] = kv
            uf[c] = jnp.dot(fm, kv, preferred_element_type=F32)
            kc = jax.lax.dot_general(fm, cs[g, :, c * C:(c + 1) * C], NT,
                                     preferred_element_type=F32) * (1.0 / C)
            if prev is None:
                kf[c] = kc
            else:
                h = C // 2
                kf[c, 0:h] = kc[0:h] - prev[C:C + h]
                kf[c, h:C] = kc[h:C] + prev[C + h:2 * C]
                kf[c, C:C + h] = kc[C:C + h] + prev[0:h]
                kf[c, C + h:2 * C] = kc[C + h:2 * C] - prev[h:C]
            prev = kc
            yield 150

    FB = 32

    def conv_mac(chunks):
        for c in chunks:
            for fb in range(C // FB):
                re = slice(fb * FB, (fb + 1) * FB)
                im = slice(C + fb * FB, C + (fb + 1) * FB)
                ar = ai = None
                for j in range(c + 1):
                    kr, ki = kf[j, re], kf[j, im]
                    ur, ui = uf[c - j, re], uf[c - j, im]
                    tr = kr * ur - ki * ui
                    ti = kr * ui + ki * ur
                    ar = tr if ar is None else ar + tr
                    ai = ti if ai is None else ai + ti
                yf[c, re] = ar.astype(BF16)
                yf[c, im] = ai.astype(BF16)
                yield 8 * (c + 1)

    def conv_inverse(g):
        lanes = pl.ds(pl.multiple_of(g * 128, 128), 128)
        dd = ssmd_ref[:, lanes].astype(F32)
        gm = gmat[...]
        for c in range(NC):
            r = slice(c * C, (c + 1) * C)
            y = jnp.dot(gm, yf[c], preferred_element_type=F32)
            ck[g, r, :] = (y + cv[g, r, :].astype(F32) * dd).astype(BF16)
            yield 80

    def first_norm(i, slot):
        rows = pl.ds(pl.multiple_of(i * BM, BM), BM)
        x = xb[rows, :].astype(F32)
        xf[rows, :] = x
        xnb[slot] = _layernorm(x).astype(BF16)

    def first_body(i, _):
        r0 = pl.multiple_of(i * BM, BM)
        for cp in c_copies(i):
            cp.wait()

        def work():
            yield from conv_forward(i)
            yield from conv_mac(range(NC))
            yield from conv_inverse(i)

        gen = work()
        done = [0]
        total = NC * (150 + 80) + (C // FB) * 8 * NC * (NC + 1) // 2

        def fill(step):
            while done[0] < total * min(step + 1, 5) // 5:
                done[0] += next(gen)
            if step == 5:
                first_norm(jnp.minimum(i + 1, NB - 1), (i + 1) % 2)

        project(xnb[i % 2], r0, fill)
        return 0

    def mix_rows(r0):
        rows = pl.ds(r0, BM)
        x = xf[rows, :] + jnp.dot(xb[rows, :], wo[...], preferred_element_type=F32)
        y = jnp.concatenate([ck[g, rows, :] for g in range(NG)], axis=1)
        return x + _layernorm(x) * y.astype(F32)

    def mid_norm(i):
        r0 = pl.multiple_of(i * BM, BM)
        x = mix_rows(r0)
        xf[pl.ds(r0, BM), :] = x
        xnb[i % 2] = _layernorm(x).astype(BF16)

    def mid_body(i, _):
        project(xnb[i % 2], pl.multiple_of(i * BM, BM),
                lambda step: mid_norm(i + 1) if step == 0 else None)
        return 0

    def last_body(i, _):
        r0 = pl.multiple_of(i * BM, BM)
        xb[pl.ds(r0, BM), :] = mix_rows(r0).astype(BF16)
        o_copy(i).start()
        return 0

    lane = jax.lax.broadcasted_iota(jnp.int32, (BQ, 128), 1)

    sbuf = (s_a, s_b)

    def masked_q(g, qb, h):
        qq = q[g, pl.ds(pl.multiple_of(qb * BQ, BQ), BQ), :]
        return jnp.where((lane >= h * DH) & (lane < (h + 1) * DH), qq, jnp.zeros_like(qq))

    def scores(g, h, c, qm, m):
        r = slice(c * BK, (c + 1) * BK)
        s = jax.lax.dot_general(k[g, r, :], qm, NT, preferred_element_type=F32)
        sbuf[h % 2][r, :] = s
        mc = s.reshape(BK // 8, 8, BQ).max(axis=0)
        return mc if m is None else jnp.maximum(m, mc)

    def attn_flush(t):
        g, qb = t // NQ, t % NQ
        xb[pl.ds(pl.multiple_of(qb * BQ, BQ), BQ),
           pl.ds(pl.multiple_of(g * 128, 128), 128)] = ot[...].T.astype(BF16)

    def attn_prologue():
        m0 = m1 = None
        qm = masked_q(0, 0, 0)
        for c in range(NKC):
            m0 = scores(0, 0, c, qm, m0)
        qm = masked_q(0, 0, 1)
        for c in range(SKEW):
            m1 = scores(0, 1, c, qm, m1)
        return jnp.max(m0, axis=0, keepdims=True), m1

    def attn_body(t, carry):
        m_done, m_run = carry
        attn_flush(jnp.maximum(t - 1, 0))
        tn = jnp.minimum(t + 1, NG * NQ - 1)
        where = ((t // NQ, t % NQ), (tn // NQ, tn % NQ))
        g = where[0][0]
        qm = masked_q(*where[0], 1)
        m_next = None
        for h in range(4):
            vrows = pl.ds(pl.multiple_of(g * 128 + h * DH, DH), DH)
            l = acc = None
            for c in range(NKC):
                ta, ca = divmod(h * NKC + c + NKC + SKEW, NKC)
                if ca == 0:
                    qm = masked_q(*where[ta // 4], ta % 4)
                m_run = scores(where[ta // 4][0], ta, ca, qm, None if ca == 0 else m_run)
                if ca == NKC - 1:
                    m_next = jnp.max(m_run, axis=0, keepdims=True)
                r = slice(c * BK, (c + 1) * BK)
                ps = []
                for u in range(BK // 16):
                    p = jnp.exp2(sbuf[h % 2][c * BK + u * 16:c * BK + u * 16 + 16, :] - m_done)
                    ps.append(p.astype(BF16))
                o = jnp.dot(jnp.concatenate([vt[vrows, r], jnp.ones((16, BK), BF16)], 0), jnp.concatenate(ps, axis=0), preferred_element_type=F32)
                acc = o if acc is None else acc + o
            ot[h * DH:(h + 1) * DH, :] = acc[:DH] / acc[DH:DH + 1]
            m_done = m_next
        return m_done, m_run

    ot[...] = jnp.zeros_like(ot)

    def layer_body(layer, _):
        @pl.when(layer == 0)
        def _():
            for i in range(NB):
                x_copy(i).wait()
            first_norm(0, 0)
            for j in range(3):
                w_copy(j).wait()
            jax.lax.fori_loop(0, NB, first_body, 0)
            w_copy(3).wait()

        jax.lax.fori_loop(0, NG * NQ, attn_body, attn_prologue())
        attn_flush(NG * NQ - 1)

        @pl.when(layer == 0)
        def _():
            mid_norm(0)
            jax.lax.fori_loop(0, NB - 1, mid_body, 0)
            project(xnb[(NB - 1) % 2], (NB - 1) * BM, lambda step: None)

        @pl.when(layer == 1)
        def _():
            jax.lax.fori_loop(0, NB, last_body, 0)

        return 0

    jax.lax.fori_loop(0, 2, layer_body, 0)
    for i in range(NB):
        o_copy(i).wait()


@jax.jit
def pallas_interleave_layers__softmax_full_mha__ssm_conv_h3__prompt_kernel(
    A_x: jax.Array,
    A_wqkv: jax.Array,
    A_wo: jax.Array,
    B_q: jax.Array,
    B_k: jax.Array,
    B_v: jax.Array,
    B_shift_k: jax.Array,
    B_ssm_k: jax.Array,
    B_ssm_D: jax.Array,
):
    del B_q
    hbm = pl.BlockSpec(memory_space=pl.ANY)
    vmem = pl.BlockSpec(memory_space=pltpu.VMEM)
    out = pl.pallas_call(
        _kernel,
        out_shape=jax.ShapeDtypeStruct((S, D), BF16),
        in_specs=[hbm, hbm, hbm, hbm, hbm, vmem, hbm, vmem],
        out_specs=hbm,
        scratch_shapes=[
            pltpu.VMEM((S, D), F32),
            pltpu.VMEM((S, D), BF16),
            pltpu.VMEM((3, D, D), BF16),
            pltpu.VMEM((D, D), BF16),
            pltpu.VMEM((NG, S, 128), BF16),
            pltpu.VMEM((NG, S, 128), BF16),
            pltpu.VMEM((D, S), BF16),
            pltpu.VMEM((S, BQ), F32),
            pltpu.VMEM((S, BQ), F32),
            pltpu.VMEM((128, BQ), F32),
            pltpu.VMEM((NG, S, 128), BF16),
            pltpu.VMEM((NG, S, 128), BF16),
            pltpu.VMEM((NG, 128, S), BF16),
            pltpu.VMEM((8 + S, 128), F32),
            pltpu.VMEM((2, BM, D), BF16),
            pltpu.VMEM((NC, 2 * C, 128), F32),
            pltpu.VMEM((NC, 2 * C, 128), F32),
            pltpu.VMEM((NC, 2 * C, 128), BF16),
            pltpu.VMEM((2 * C, C), BF16),
            pltpu.VMEM((C, 2 * C), BF16),
            pltpu.SemaphoreType.DMA((NB,)),
            pltpu.SemaphoreType.DMA((4,)),
            pltpu.SemaphoreType.DMA((3 * NG,)),
            pltpu.SemaphoreType.DMA((NB,)),
        ],
        compiler_params=pltpu.CompilerParams(vmem_limit_bytes=100 * 2**20),
    )(A_x.reshape(S, D), A_wqkv, A_wo, B_k.reshape(S, D), B_v.reshape(S, D),
      B_shift_k.T, B_ssm_k, B_ssm_D.reshape(1, D))
    return out.reshape(1, S, D)
```

```python
import math

import jax
import jax.numpy as jnp
import jax.experimental.pallas as pl
import jax.experimental.pallas.tpu as pltpu

F32 = jnp.float32
BF16 = jnp.bfloat16

S = 2048
D = 1024
DH = 32
NG = D // 128
BM = 256
NB = S // BM
BQ = 512
BK = 128
NQ = S // BQ
NKC = S // BK
SKEW = 2
C = 128
NC = S // C
EPS = 1e-5
Q_SCALE = DH ** -0.5 * math.log2(math.e)

NT = (((1,), (1,)), ((), ()))


def _layernorm(x):
    m = jnp.mean(x, axis=-1, keepdims=True)
    xc = x - m
    v = jnp.mean(xc * xc, axis=-1, keepdims=True)
    return xc * jax.lax.rsqrt(v + EPS)


def _kernel(x_hbm, wqkv_hbm, wo_hbm, bk_hbm, bv_hbm, sk_ref, ssmk_hbm, ssmd_ref,
            out_hbm,
            xf, xb, wqkv, wo, q, k, vt, s_a, s_b, ot, ck, cv, cs, kpad,
            xnb, uf, kf, yf, fmat, gmat, sem_x, sem_w, sem_c, sem_o):

    def x_copy(i):
        r = pl.ds(i * BM, BM)
        return pltpu.make_async_copy(x_hbm.at[r], xb.at[r], sem_x.at[i])

    def w_copy(j):
        if j < 3:
            c = pl.ds(j * D, D)
            return pltpu.make_async_copy(wqkv_hbm.at[:, c], wqkv.at[j], sem_w.at[j])
        return pltpu.make_async_copy(wo_hbm, wo, sem_w.at[3])

    def c_copies(g):
        c = pl.ds(g * 128, 128)
        return (pltpu.make_async_copy(bk_hbm.at[:, c], ck.at[g], sem_c.at[3 * g]),
                pltpu.make_async_copy(bv_hbm.at[:, c], cv.at[g], sem_c.at[3 * g + 1]),
                pltpu.make_async_copy(ssmk_hbm.at[c], cs.at[g], sem_c.at[3 * g + 2]))

    def o_copy(i):
        r = pl.ds(i * BM, BM)
        return pltpu.make_async_copy(xb.at[r], out_hbm.at[r], sem_o.at[i])

    for i in range(NB):
        x_copy(i).start()
    for j in range(3):
        w_copy(j).start()
    for i in range(NB):
        for cp in c_copies(i):
            cp.start()
    w_copy(3).start()

    row = jax.lax.broadcasted_iota(jnp.int32, (C, C), 0)
    col = jax.lax.broadcasted_iota(jnp.int32, (C, C), 1)

    def twiddle(r, t):
        f = jnp.where(r < C // 2, 2 * r, 2 * r - (C - 1))
        ph = (((2 * f + 1) * t) & (4 * C - 1)).astype(F32) * (2 * math.pi / (4 * C))
        return jnp.cos(ph), -jnp.sin(ph)

    cr, ci = twiddle(row, col)
    fmat[0:C, :] = cr.astype(BF16)
    fmat[C:2 * C, :] = ci.astype(BF16)
    cr, ci = twiddle(col, row)
    gmat[:, 0:C] = cr.astype(BF16)
    gmat[:, C:2 * C] = ci.astype(BF16)
    kpad[0:8, :] = jnp.zeros((8, 128), F32)

    def project(xn, r0, fill):
        for j in range(3):
            for n in range(2):
                y = jnp.dot(xn, wqkv[j, :, n * 512:(n + 1) * 512], preferred_element_type=F32)
                if j == 2:
                    vt[n * 512:(n + 1) * 512, pl.ds(r0, BM)] = y.T.astype(BF16)
                else:
                    y = (y * Q_SCALE if j == 0 else y).astype(BF16)
                    for g in range(4):
                        (q, k)[j][4 * n + g, pl.ds(r0, BM), :] = y[:, g * 128:(g + 1) * 128]
                fill(2 * j + n)

    def conv_forward(g):
        lanes = pl.ds(pl.multiple_of(g * 128, 128), 128)
        sk = sk_ref[:, lanes].astype(F32)
        kpad[8:8 + S, :] = ck[g].astype(F32)
        fm = fmat[...]
        prev = None
        for c in range(NC):
            ks = kpad[8 + c * C:8 + (c + 1) * C, :] * sk[0:1]
            for j in range(1, 4):
                ks = ks + kpad[8 - j + c * C:8 - j + (c + 1) * C, :] * sk[j:j + 1]
            kv = (ks * cv[g, c * C:(c + 1) * C, :].astype(F32)).astype(BF16)
            cv[g, c * C:(c + 1) * C, :] = kv
            uf[c] = jnp.dot(fm, kv, preferred_element_type=F32)
            kc = jax.lax.dot_general(fm, cs[g, :, c * C:(c + 1) * C], NT,
                                     preferred_element_type=F32) * (1.0 / C)
            if prev is None:
                kf[c] = kc
            else:
                h = C // 2
                kf[c, 0:h] = kc[0:h] - prev[C:C + h]
                kf[c, h:C] = kc[h:C] + prev[C + h:2 * C]
                kf[c, C:C + h] = kc[C:C + h] + prev[0:h]
                kf[c, C + h:2 * C] = kc[C + h:2 * C] - prev[h:C]
            prev = kc
            yield 150

    FB = 32

    def conv_mac(chunks):
        for c in chunks:
            for fb in range(C // FB):
                re = slice(fb * FB, (fb + 1) * FB)
                im = slice(C + fb * FB, C + (fb + 1) * FB)
                ar = ai = None
                for j in range(c + 1):
                    kr, ki = kf[j, re], kf[j, im]
                    ur, ui = uf[c - j, re], uf[c - j, im]
                    tr = kr * ur - ki * ui
                    ti = kr * ui + ki * ur
                    ar = tr if ar is None else ar + tr
                    ai = ti if ai is None else ai + ti
                yf[c, re] = ar.astype(BF16)
                yf[c, im] = ai.astype(BF16)
                yield 8 * (c + 1)

    def conv_inverse(g):
        lanes = pl.ds(pl.multiple_of(g * 128, 128), 128)
        dd = ssmd_ref[:, lanes].astype(F32)
        gm = gmat[...]
        for c in range(NC):
            r = slice(c * C, (c + 1) * C)
            y = jnp.dot(gm, yf[c], preferred_element_type=F32)
            ck[g, r, :] = (y + cv[g, r, :].astype(F32) * dd).astype(BF16)
            yield 80

    def first_norm(i, slot):
        rows = pl.ds(pl.multiple_of(i * BM, BM), BM)
        x = xb[rows, :].astype(F32)
        xf[rows, :] = x
        xnb[slot] = _layernorm(x).astype(BF16)

    def first_body(i, _):
        r0 = pl.multiple_of(i * BM, BM)
        for cp in c_copies(i):
            cp.wait()

        def fill(step):
            if step == 5:
                first_norm(jnp.minimum(i + 1, NB - 1), (i + 1) % 2)
                return
            stage = (conv_forward(i) if step == 0 else conv_inverse(i) if step == 4 else
                     conv_mac((range(0, 9), range(9, 13), range(13, NC))[step - 1]))
            for _ in stage:
                pass

        project(xnb[i % 2], r0, fill)
        return 0

    def mix_rows(r0):
        rows = pl.ds(r0, BM)
        x = xf[rows, :] + jnp.dot(xb[rows, :], wo[...], preferred_element_type=F32)
        y = jnp.concatenate([ck[g, rows, :] for g in range(NG)], axis=1)
        return x + _layernorm(x) * y.astype(F32)

    def mid_norm(i):
        r0 = pl.multiple_of(i * BM, BM)
        x = mix_rows(r0)
        xf[pl.ds(r0, BM), :] = x
        xnb[i % 2] = _layernorm(x).astype(BF16)

    def mid_body(i, _):
        project(xnb[i % 2], pl.multiple_of(i * BM, BM),
                lambda step: mid_norm(i + 1) if step == 0 else None)
        return 0

    def last_body(i, _):
        r0 = pl.multiple_of(i * BM, BM)
        xb[pl.ds(r0, BM), :] = mix_rows(r0).astype(BF16)
        o_copy(i).start()
        return 0

    lane = jax.lax.broadcasted_iota(jnp.int32, (BQ, 128), 1)

    sbuf = (s_a, s_b)

    def masked_q(g, qb, h):
        qq = q[g, pl.ds(pl.multiple_of(qb * BQ, BQ), BQ), :]
        return jnp.where((lane >= h * DH) & (lane < (h + 1) * DH), qq, jnp.zeros_like(qq))

    def scores(g, h, c, qm, m):
        r = slice(c * BK, (c + 1) * BK)
        s = jax.lax.dot_general(k[g, r, :], qm, NT, preferred_element_type=F32)
        sbuf[h % 2][r, :] = s
        mc = s.reshape(BK // 8, 8, BQ).max(axis=0)
        return mc if m is None else jnp.maximum(m, mc)

    def attn_flush(t):
        g, qb = t // NQ, t % NQ
        xb[pl.ds(pl.multiple_of(qb * BQ, BQ), BQ),
           pl.ds(pl.multiple_of(g * 128, 128), 128)] = ot[...].T.astype(BF16)

    def attn_prologue():
        m0 = m1 = None
        qm = masked_q(0, 0, 0)
        for c in range(NKC):
            m0 = scores(0, 0, c, qm, m0)
        qm = masked_q(0, 0, 1)
        for c in range(SKEW):
            m1 = scores(0, 1, c, qm, m1)
        return jnp.max(m0, axis=0, keepdims=True), m1

    def attn_body(t, carry):
        m_done, m_run = carry
        attn_flush(jnp.maximum(t - 1, 0))
        tn = jnp.minimum(t + 1, NG * NQ - 1)
        where = ((t // NQ, t % NQ), (tn // NQ, tn % NQ))
        g = where[0][0]
        qm = masked_q(*where[0], 1)
        m_next = None
        for h in range(4):
            vrows = pl.ds(pl.multiple_of(g * 128 + h * DH, DH), DH)
            l = acc = None
            for c in range(NKC):
                ta, ca = divmod(h * NKC + c + NKC + SKEW, NKC)
                if ca == 0:
                    qm = masked_q(*where[ta // 4], ta % 4)
                m_run = scores(where[ta // 4][0], ta, ca, qm, None if ca == 0 else m_run)
                if ca == NKC - 1:
                    m_next = jnp.max(m_run, axis=0, keepdims=True)
                r = slice(c * BK, (c + 1) * BK)
                ps = []
                for u in range(BK // 16):
                    p = jnp.exp2(sbuf[h % 2][c * BK + u * 16:c * BK + u * 16 + 16, :] - m_done)
                    ps.append(p.astype(BF16))
                o = jnp.dot(jnp.concatenate([vt[vrows, r], jnp.ones((16, BK), BF16)], 0), jnp.concatenate(ps, axis=0), preferred_element_type=F32)
                acc = o if acc is None else acc + o
            ot[h * DH:(h + 1) * DH, :] = acc[:DH] / acc[DH:DH + 1]
            m_done = m_next
        return m_done, m_run

    ot[...] = jnp.zeros_like(ot)

    def layer_body(layer, _):
        @pl.when(layer == 0)
        def _():
            for i in range(NB):
                x_copy(i).wait()
            first_norm(0, 0)
            for j in range(3):
                w_copy(j).wait()
            jax.lax.fori_loop(0, NB, first_body, 0)
            w_copy(3).wait()

        jax.lax.fori_loop(0, NG * NQ, attn_body, attn_prologue())
        attn_flush(NG * NQ - 1)

        @pl.when(layer == 0)
        def _():
            mid_norm(0)
            jax.lax.fori_loop(0, NB - 1, mid_body, 0)
            project(xnb[(NB - 1) % 2], (NB - 1) * BM, lambda step: None)

        @pl.when(layer == 1)
        def _():
            jax.lax.fori_loop(0, NB, last_body, 0)

        return 0

    jax.lax.fori_loop(0, 2, layer_body, 0)
    for i in range(NB):
        o_copy(i).wait()


@jax.jit
def pallas_interleave_layers__softmax_full_mha__ssm_conv_h3__prompt_kernel(
    A_x: jax.Array,
    A_wqkv: jax.Array,
    A_wo: jax.Array,
    B_q: jax.Array,
    B_k: jax.Array,
    B_v: jax.Array,
    B_shift_k: jax.Array,
    B_ssm_k: jax.Array,
    B_ssm_D: jax.Array,
):
    del B_q
    hbm = pl.BlockSpec(memory_space=pl.ANY)
    vmem = pl.BlockSpec(memory_space=pltpu.VMEM)
    out = pl.pallas_call(
        _kernel,
        out_shape=jax.ShapeDtypeStruct((S, D), BF16),
        in_specs=[hbm, hbm, hbm, hbm, hbm, vmem, hbm, vmem],
        out_specs=hbm,
        scratch_shapes=[
            pltpu.VMEM((S, D), F32),
            pltpu.VMEM((S, D), BF16),
            pltpu.VMEM((3, D, D), BF16),
            pltpu.VMEM((D, D), BF16),
            pltpu.VMEM((NG, S, 128), BF16),
            pltpu.VMEM((NG, S, 128), BF16),
            pltpu.VMEM((D, S), BF16),
            pltpu.VMEM((S, BQ), F32),
            pltpu.VMEM((S, BQ), F32),
            pltpu.VMEM((128, BQ), F32),
            pltpu.VMEM((NG, S, 128), BF16),
            pltpu.VMEM((NG, S, 128), BF16),
            pltpu.VMEM((NG, 128, S), BF16),
            pltpu.VMEM((8 + S, 128), F32),
            pltpu.VMEM((2, BM, D), BF16),
            pltpu.VMEM((NC, 2 * C, 128), F32),
            pltpu.VMEM((NC, 2 * C, 128), F32),
            pltpu.VMEM((NC, 2 * C, 128), BF16),
            pltpu.VMEM((2 * C, C), BF16),
            pltpu.VMEM((C, 2 * C), BF16),
            pltpu.SemaphoreType.DMA((NB,)),
            pltpu.SemaphoreType.DMA((4,)),
            pltpu.SemaphoreType.DMA((3 * NG,)),
            pltpu.SemaphoreType.DMA((NB,)),
        ],
        compiler_params=pltpu.CompilerParams(vmem_limit_bytes=100 * 2**20),
    )(A_x.reshape(S, D), A_wqkv, A_wo, B_k.reshape(S, D), B_v.reshape(S, D),
      B_shift_k.T, B_ssm_k, B_ssm_D.reshape(1, D))
    return out.reshape(1, S, D)
```
